```python
import jax
import jax.numpy as jnp

def _softmax(x, axis=-1):
    return jax.nn.softmax(x, axis=axis)
def _gelu(x):
    return jax.nn.gelu(x, approximate=True)
def _silu(x):
    return jax.nn.silu(x)
def _sigmoid(x):
    return jax.nn.sigmoid(x)
def _layernorm(x, axis=-1, eps=1e-5):
    m = jnp.mean(x, axis=axis, keepdims=True)
    v = jnp.var(x, axis=axis, keepdims=True)
    return (x - m) / jnp.sqrt(v + eps)
def _scatter_add(tgt, idx, src, axis=0):
    return tgt.at[idx].add(src)
def _segment_sum(src, seg, n):
    return jax.ops.segment_sum(src, seg, n)
class _Rng:
    def __init__(self, key):
        self._k = key
    def _next(self):
        self._k, sub = jax.random.split(self._k)
        return sub
    def normal(self, shape):
        return jax.random.normal(self._next(), shape, dtype=jnp.bfloat16)
    def randint(self, lo, hi, shape):
        return jax.random.randint(self._next(), shape, lo, hi, dtype=jnp.int32)
    def uniform(self, shape, lo=0.0, hi=1.0):
        return jax.random.uniform(self._next(), shape, jnp.bfloat16, lo, hi)
    def permutation(self, n):
        return jax.random.permutation(self._next(), n)


kernel_name = 'recurrent_scan__sliding_block_cached__mixer_s_mlp__decode'

def _fwd_setup_inputs():
    _rng = _Rng(jax.random.key(int.from_bytes(__import__("os").urandom(4), "little")))
    _w = (lambda a: (lambda t: t.astype(jnp.bfloat16) if jnp.issubdtype(t.dtype, jnp.floating) else t)(jnp.asarray(a)))
    def _A_setup():
        B, Sq, D = 4, 1, 512
        Hq, Hkv, Sk, Dh = 32, 8, 8192, 128
        assert Hq % Hkv == 0, (Hq, Hkv)
        return {
            "x": _w((lambda *s: _rng.normal(s) * 0.05)(B, Sq, D)),
            "k_cache": _w((lambda *s: _rng.normal(s) * 0.05)(B, Hkv, Sk, Dh)),
            "v_cache": _w((lambda *s: _rng.normal(s) * 0.05)(B, Hkv, Sk, Dh)),
            "wq": _w((lambda *s: _rng.normal(s) * 0.05)(D, Hq * Dh) * (D ** -0.5)),
            "wo": _w((lambda *s: _rng.normal(s) * 0.05)(Hq * Dh, D) * ((Hq * Dh) ** -0.5)),
        }
    _A_in = _A_setup()

    def _B_setup():
        B, S, D, F = 4, 1, 512, 1792
        return {
            "x":  _w((lambda *s: _rng.normal(s) * 0.05)(B, S, D)),
            "w1": _w((lambda *s: _rng.normal(s) * 0.05)(D, D) * (D ** -0.5)),
            "w2": _w((lambda *s: _rng.normal(s) * 0.05)(D, D) * (D ** -0.5)),
            "w3": _w((lambda *s: _rng.normal(s) * 0.05)(D, F) * (D ** -0.5)),
            "w4": _w((lambda *s: _rng.normal(s) * 0.05)(F, D) * (F ** -0.5)),
        }
    _B_in = _B_setup()

    return {
        "A_x": _A_in["x"],
        "A_k_cache": _A_in["k_cache"],
        "A_v_cache": _A_in["v_cache"],
        "A_wq": _A_in["wq"],
        "A_wo": _A_in["wo"],
        "B_x": _B_in["x"],
        "B_w1": _B_in["w1"],
        "B_w2": _B_in["w2"],
        "B_w3": _B_in["w3"],
        "B_w4": _B_in["w4"],
    }

def _fwd_reference(A_x, A_k_cache, A_v_cache, A_wq, A_wo, B_x, B_w1, B_w2, B_w3, B_w4):
    def _A_ref(x, k_cache, v_cache, wq, wo):
        B, Sq, D = x.shape
        Hq, Dh = 32, 128
        Hkv, Sk = k_cache.shape[1], k_cache.shape[2]
        W = min(4096, max(256, Sk // 4))
        rep = Hq // Hkv
        q = (lambda x, *d: x.transpose(*d))((x @ wq).reshape(B, Sq, Hq, Dh), 0, 2, 1, 3)
        k = jnp.repeat(k_cache[:, :, Sk - W:, :], rep, axis=1)
        v = jnp.repeat(v_cache[:, :, Sk - W:, :], rep, axis=1)
        scores = jnp.einsum("bhqd,bhkd->bhqk", q, k) * (Dh ** -0.5)
        p = _softmax(scores, axis=-1)
        o = jnp.einsum("bhqk,bhkd->bhqd", p, v)
        return (lambda x, *d: x.transpose(*d))(o, 0, 2, 1, 3).reshape(B, Sq, Hq * Dh) @ wo

    def _B_ref(x, w1, w2, w3, w4):
        B, S, D = x.shape
        h = _gelu(_layernorm(x, axis=-1) @ w1)
        c = D // 4
        g0 = jnp.pad(h[:, :, 0*c:1*c], ((0, 0), (1, 0), (0, 0)))[:, :S, :]
        g1 = jnp.pad(h[:, :, 1*c:2*c], ((0, 0), (0, 1), (0, 0)))[:, 1:, :]
        g2 = jnp.pad(h[:, :, 2*c:3*c], ((0, 0), (2, 0), (0, 0)))[:, :S, :]
        g3 = jnp.pad(h[:, :, 3*c:   ], ((0, 0), (0, 2), (0, 0)))[:, 2:, :]
        hs = jnp.concatenate([g0, g1, g2, g3], axis=-1) @ w2
        x1 = x + hs
        h2 = _gelu(_layernorm(x1, axis=-1) @ w3) @ w4
        return x1 + h2

    x = A_x
    xn = _layernorm(x, axis=-1)
    s = _A_ref(xn, A_k_cache, A_v_cache, A_wq, A_wo)
    g = _silu(_B_ref(xn, B_w1, B_w2, B_w3, B_w4))
    return x + s * g


def setup_inputs():
    _inp = _fwd_setup_inputs()
    _gk = jax.random.fold_in(jax.random.key(int.from_bytes(__import__("os").urandom(4), "little")), 2**31 - 1)
    _shapes = [[4, 1, 512]]
    _dtypes = ['bfloat16']
    _gks = jax.random.split(_gk, len(_shapes))
    _gs = [jax.random.normal(k, s, dtype=jnp.dtype(d)) * 0.05 for k, s, d in zip(_gks, _shapes, _dtypes)]
    _inp["grad_out"] = _gs[0]
    return _inp

def reference(A_x, A_k_cache, A_v_cache, A_wq, A_wo, B_w3, B_w4, B_x, B_w1, B_w2, grad_out):
    _const = dict(B_x=B_x, B_w1=B_w1, B_w2=B_w2)
    def _f(*_d):
        return _fwd_reference(**{'A_x': _d[0], 'A_k_cache': _d[1], 'A_v_cache': _d[2], 'A_wq': _d[3], 'A_wo': _d[4], 'B_w3': _d[5], 'B_w4': _d[6], **_const})
    _out, _vjp = jax.vjp(_f, A_x, A_k_cache, A_v_cache, A_wq, A_wo, B_w3, B_w4)
    _grads = _vjp(grad_out)
    _out0 = jnp.asarray(_out)
    return (_out0, *[jnp.asarray(_g) for _g in _grads])
```

```python
import functools

import jax
import jax.numpy as jnp
from jax import lax
import jax.experimental.pallas as pl
import jax.experimental.pallas.tpu as pltpu

B, D, F = 4, 512, 1792
HQ, HKV, SK, DH = 32, 8, 8192, 128
REP = HQ // HKV
W = min(4096, max(256, SK // 4))
W0 = SK - W
EPS = 1e-5
BF = jnp.bfloat16
F32 = jnp.float32

NN = (((1,), (0,)), ((), ()))
NT = (((1,), (1,)), ((), ()))
TN = (((0,), (0,)), ((), ()))


def _dot(a, b, dims=NN):
  return lax.dot_general(a.astype(BF), b, dims, preferred_element_type=F32)


def _ln(x):
  xc = x - jnp.mean(x, axis=-1, keepdims=True)
  var = jnp.mean(xc * xc, axis=-1, keepdims=True)
  rstd = 1.0 / jnp.sqrt(var + EPS)
  return xc * rstd, rstd


def _ln_bwd(dy, xhat, rstd):
  return rstd * (dy - jnp.mean(dy, axis=-1, keepdims=True)
                 - xhat * jnp.mean(dy * xhat, axis=-1, keepdims=True))


_C0 = 0.7978845608028654
_C1 = 0.044715


def _gelu_and_grad(x):
  x2 = x * x
  t = jnp.tanh(_C0 * (x + _C1 * x * x2))
  cdf = 0.5 * (1.0 + t)
  return x * cdf, cdf + x * (0.5 * (1.0 - t * t)) * (_C0 * (1.0 + 3.0 * _C1 * x2))


def make(rpat='0111', rdepth=64, wrows=64, early=8, zper=24, zpre=64, compute=True,
         scopes=False, nobounds=True, kv_inter=False):
  RC = 64
  NS = 16
  cpi = rdepth // NS
  NZC = W0 // wrows
  NDC = W // wrows

  def scope(name):
    return jax.named_scope(name) if scopes else _Null()

  def kernel(x_hbm, k_hbm, v_hbm, wq_hbm, wo_hbm, w3_hbm, w4_hbm, go_hbm,
             out_hbm, dx_hbm, dk_hbm, dv_hbm, dwq_hbm, dwo_hbm, dw3_hbm, dw4_hbm,
             kbuf, vbuf, wq, wo, w3, w4, dwq, dwo, dw3, dw4, zbuf,
             xs, gos, outs, dxs, q_s, do_s, o_s, dq_s,
             rsem, ssem, wsem):

    def rd(src, dst, j):
      pltpu.make_async_copy(src, dst, rsem.at[j]).start(priority=int(rpat[j % len(rpat)]))

    def rwait(j):
      ref = kbuf.at[0, 0, pl.ds(0, RC)]
      pltpu.make_async_copy(ref, ref, rsem.at[j]).wait()

    def rd_w34(c0, j):
      s, c = j % NS, c0 + j // NS
      if s % 2 == 0:
        idx = (pl.ds((s // 2) * 64 + (c // 7) * 32, 32), pl.ds((c % 7) * 256, 256))
        rd(w3_hbm.at[idx], w3.at[idx], j)
      else:
        idx = (pl.ds((s // 2) * 224 + c * 16, 16), slice(None))
        rd(w4_hbm.at[idx], w4.at[idx], j)

    def rd_wqo(i, j):
      s, cc = j % NS, j // NS
      if s % 2 == 0:
        c = i * cpi + cc
        r = pl.multiple_of((s // 2) * 64 + (c >> 3) * 16, 16)
        col = pl.multiple_of((c & 7) * 512, 512)
        idx = (pl.ds(r, 16), pl.ds(col, 512))
        rd(wq_hbm.at[idx], wq.at[idx], j)
      else:
        r = pl.multiple_of((s // 2) * 512 + (i * cpi + cc) * 16, 16)
        idx = (pl.ds(r, 16), slice(None))
        rd(wo_hbm.at[idx], wo.at[idx], j)

    ipb = (W // RC) // cpi

    def rd_kv(i, j):
      s, cc = j % NS, j // NS
      b = i // ipb if isinstance(i, int) else lax.div(i, ipb)
      r = ((i - b * ipb) * cpi + cc) * RC
      if kv_inter:
        src, dst, h = ((k_hbm, kbuf), (v_hbm, vbuf))[s % 2] + (s // 2,)
      else:
        src, dst, h = ((k_hbm, kbuf), (v_hbm, vbuf))[s // 8] + (s % 8,)
      rd(src.at[b, h, pl.ds(pl.multiple_of(W0 + r, RC), RC)],
         dst.at[b, h, pl.ds(pl.multiple_of(r, RC), RC)], j)

    cp_x = pltpu.make_async_copy(x_hbm, xs, ssem.at[0])
    cp_go = pltpu.make_async_copy(go_hbm, gos, ssem.at[1])

    with scope("reads"):
      n34 = 14 * NS
      for t in range(n34):
        j = t % rdepth
        if t >= rdepth:
          rwait(j)
        rd_w34((t // rdepth) * cpi, j)
        if t == rdepth - 1:
          cp_x.start()
          cp_go.start()
          zbuf[...] = jnp.zeros(zbuf.shape, BF)
      rot = n34 % rdepth

      def wqo_body(i, _):
        for t in range(rdepth):
          j = (t + rot) % rdepth
          rwait(j)
          rd_wqo(i, j)
      lax.fori_loop(0, 32 // cpi, wqo_body, None)

      def kv_body(i, _):
        for t in range(rdepth):
          j = (t + rot) % rdepth
          rwait(j)
          rd_kv(i, j)
      lax.fori_loop(0, B * ipb, kv_body, None)

      for t in range(rdepth - early):
        rwait((t + rot) % rdepth)

    def zero_fill(i):
      g = i // NZC if isinstance(i, int) else lax.div(i, NZC)
      r = pl.multiple_of((i - g * NZC) * wrows, wrows)
      return g, r

    def zero_range(lo, n):
      def body(t, _):
        g, r = zero_fill(t)

        @pl.when(g < B)
        def _():
          pltpu.make_async_copy(zbuf, dk_hbm.at[g, :, pl.ds(r, wrows)], wsem.at[0]).start()

        @pl.when(g >= B)
        def _():
          pltpu.make_async_copy(zbuf, dv_hbm.at[g - B, :, pl.ds(r, wrows)], wsem.at[1]).start()
      lax.fori_loop(lo, lo + n, body, None)

    NZ = 2 * B * NZC
    zero_range(0, 2)
    for t in range(rdepth - early, rdepth):
      rwait((t + rot) % rdepth)
    cp_x.wait()
    cp_go.wait()
    zero_range(2, zpre - 2)
    zpos = zpre

    if compute:
      pad = jnp.zeros((8 - B, D), F32)
      x = jnp.concatenate([xs[...].astype(F32), pad], axis=0)
      go = jnp.concatenate([gos[...].astype(F32), pad], axis=0)
      xhat, rstd1 = _ln(x)
      xn = xhat
      ln2, rstd2 = _ln(xn)
      pre = _dot(ln2, w3[...])
      hh, dgelu = _gelu_and_grad(pre)
      bo = xn + _dot(hh, w4[...])
      sig = jax.nn.sigmoid(bo)
      g = bo * sig
      ds = go * g

      def spread(ref, val):
        for j in range(HQ):
          tile = val[:B, j * DH:(j + 1) * DH]
          r0 = (j // REP) * 8 + j % REP
          ref[pl.ds(r0, B, stride=8 * HKV), :] = tile
          ref[pl.ds(r0 + REP, B, stride=8 * HKV), :] = tile

      spread(q_s, _dot(xn, wq[...]))
      zero_range(zpos, zper)
      zpos += zper
      spread(do_s, _dot(ds, wo[...], NT))

    scale = DH ** -0.5
    zleft = NZ - zpos - 2 * zper
    zloop = zleft // (B * HKV)

    def pair(i, _):
      zero_range(zpos + i * zloop, zloop)
      if compute:
        b = i >> 3
        h = i & 7
        r = pl.multiple_of(i * 8, 8)
        q8 = q_s[pl.ds(r, 8), :]
        do8 = do_s[pl.ds(r, 8), :]
        k = kbuf[b, h]
        v = vbuf[b, h]
        s = _dot(q8, k, NT) * scale
        e = jnp.exp(s - jnp.max(s, axis=-1, keepdims=True))
        p = e / jnp.sum(e, axis=-1, keepdims=True)
        dp = _dot(do8, v, NT)
        dsc = p * (dp - jnp.sum(p * dp, axis=-1, keepdims=True)) * scale
        o_s[pl.ds(r, 8), :] = _dot(p, v)
        dq_s[pl.ds(r, 8), :] = _dot(dsc, k)
        low = lax.broadcasted_iota(jnp.int32, (8, W), 0) < REP
        t = jnp.where(low, dsc, p)
        low = lax.broadcasted_iota(jnp.int32, (8, DH), 0) < REP
        rhs = jnp.concatenate([jnp.where(low, q8, 0.0), jnp.where(low, 0.0, do8)], axis=1)
        d = _dot(t.T, rhs.astype(BF)).astype(BF)
        kbuf[b, h] = d[:, :DH]
        vbuf[b, h] = d[:, DH:]

    with scope("pairs"):
      lax.fori_loop(0, B * HKV, pair, None)
    zpos += zloop * B * HKV

    zero_range(zpos, zper)
    zpos += zper
    if compute:
      zrow = jnp.zeros((8 - B, DH), F32)

      def gather(ref):
        tiles = []
        for j in range(HQ):
          r0 = (j // REP) * 8 + j % REP
          tiles.append(jnp.concatenate([ref[pl.ds(r0, B, stride=8 * HKV), :], zrow], axis=0))
        return jnp.concatenate(tiles, axis=1)

      o = gather(o_s)
      dq = gather(dq_s)
      s = _dot(o, wo[...])
      out = x + s * g
      outs[...] = out[:B].astype(BF)
      db = go * s * (sig * (1.0 + bo * (1.0 - sig)))
      dpre = _dot(db, w4[...], NT) * dgelu
      dxn = db + _ln_bwd(_dot(dpre, w3[...], NT), ln2, rstd2) + _dot(dq, wq[...], NT)
      dx = go + _ln_bwd(dxn, xhat, rstd1)
      dxs[...] = dx[:B].astype(BF)
      dw3[...] = _dot(ln2.T, dpre.astype(BF)).astype(BF)
      dw4[...] = _dot(hh.T, db.astype(BF)).astype(BF)
    else:
      outs[...] = jnp.zeros(outs.shape, BF)
      dxs[...] = jnp.zeros(outs.shape, BF)

    zero_range(zpos, NZ - zpos)
    cp_out = pltpu.make_async_copy(outs, out_hbm, ssem.at[0])
    cp_dx = pltpu.make_async_copy(dxs, dx_hbm, ssem.at[1])
    cp_out.start()
    cp_dx.start()

    def data_range(buf, hbm, sem, extra):
      def body(t, _):
        b = lax.div(t, NDC)
        r = pl.multiple_of((t - b * NDC) * wrows, wrows)
        pltpu.make_async_copy(buf.at[b, :, pl.ds(r, wrows)],
                              hbm.at[b, :, pl.ds(pl.multiple_of(W0 + r, wrows), wrows)], sem).start()
        extra(t)
      lax.fori_loop(0, B * NDC, body, None)

    def dw4_piece(t):
      @pl.when(t < F // 16)
      def _():
        idx = (pl.ds(pl.multiple_of(t * 16, 16), 16), slice(None))
        pltpu.make_async_copy(dw4.at[idx], dw4_hbm.at[idx], wsem.at[5]).start()

    def dw3_piece(t):
      @pl.when(t < F // 16)
      def _():
        band = lax.div(t, 7)
        idx = (pl.ds(pl.multiple_of(band * 32, 32), 32), pl.ds(pl.multiple_of((t - band * 7) * 256, 256), 256))
        pltpu.make_async_copy(dw3.at[idx], dw3_hbm.at[idx], wsem.at[4]).start()

    data_range(kbuf, dk_hbm, wsem.at[0], dw4_piece)
    if compute:
      dwq[...] = _dot(xn.T, dq.astype(BF)).astype(BF)
      dwo[...] = _dot(o.T, ds.astype(BF)).astype(BF)
    data_range(vbuf, dv_hbm, wsem.at[1], dw3_piece)

    dwq3, dwq3_hbm = dwq.reshape(8, 64, HQ * DH), dwq_hbm.reshape(8, 64, HQ * DH)
    dwo3, dwo3_hbm = dwo.reshape(8, 512, D), dwo_hbm.reshape(8, 512, D)

    def dwq_body(c, _):
      idx = (slice(None), pl.ds(pl.multiple_of((c >> 3) * 16, 16), 16), pl.ds(pl.multiple_of((c & 7) * 512, 512), 512))
      pltpu.make_async_copy(dwq3.at[idx], dwq3_hbm.at[idx], wsem.at[2]).start()
    lax.fori_loop(0, 32, dwq_body, None)

    def dwo_body(c, _):
      idx = (slice(None), pl.ds(pl.multiple_of(c * 16, 16), 16), slice(None))
      pltpu.make_async_copy(dwo3.at[idx], dwo3_hbm.at[idx], wsem.at[3]).start()
    lax.fori_loop(0, 32, dwo_body, None)

    with scope("drain"):
      cp_out.wait()
      cp_dx.wait()
      for n, ref in enumerate((dk_hbm, dv_hbm, dwq_hbm, dwo_hbm, dw3_hbm, dw4_hbm)):
        pltpu.make_async_copy(ref, ref, wsem.at[n]).wait()

  hbm = pl.BlockSpec(memory_space=pltpu.HBM)
  sds = jax.ShapeDtypeStruct
  call = pl.pallas_call(
      kernel,
      out_shape=(sds((B, D), BF), sds((B, D), BF),
                 sds((B, HKV, SK, DH), BF), sds((B, HKV, SK, DH), BF),
                 sds((D, HQ * DH), BF), sds((HQ * DH, D), BF), sds((D, F), BF), sds((F, D), BF)),
      in_specs=[hbm] * 8,
      out_specs=(hbm,) * 8,
      scratch_shapes=[
          pltpu.VMEM((B, HKV, W, DH), BF), pltpu.VMEM((B, HKV, W, DH), BF),
          pltpu.VMEM((D, HQ * DH), BF), pltpu.VMEM((HQ * DH, D), BF), pltpu.VMEM((D, F), BF), pltpu.VMEM((F, D), BF),
          pltpu.VMEM((D, HQ * DH), BF), pltpu.VMEM((HQ * DH, D), BF), pltpu.VMEM((D, F), BF), pltpu.VMEM((F, D), BF),
          pltpu.VMEM((HKV, wrows, DH), BF),
          pltpu.VMEM((B, D), BF), pltpu.VMEM((B, D), BF), pltpu.VMEM((B, D), BF), pltpu.VMEM((B, D), BF),
          pltpu.VMEM((B * HKV * 8, DH), F32), pltpu.VMEM((B * HKV * 8, DH), F32),
          pltpu.VMEM((B * HKV * 8, DH), F32), pltpu.VMEM((B * HKV * 8, DH), F32),
          pltpu.SemaphoreType.DMA((rdepth,)), pltpu.SemaphoreType.DMA((2,)), pltpu.SemaphoreType.DMA((6,)),
      ],
      compiler_params=pltpu.CompilerParams(vmem_limit_bytes=100 << 20, disable_bounds_checks=nobounds),
  )

  @jax.jit
  def fn(A_x, A_k_cache, A_v_cache, A_wq, A_wo, B_x, B_w1, B_w2, B_w3, B_w4, grad_out):
    out, dx, *grads = call(A_x.reshape(B, D), A_k_cache, A_v_cache, A_wq, A_wo, B_w3, B_w4, grad_out.reshape(B, D))
    return (out.reshape(B, 1, D), dx.reshape(B, 1, D), *grads)

  return fn


class _Null:
  def __enter__(self):
    return None

  def __exit__(self, *a):
    return False


_fn = make()


@jax.jit
def pallas_recurrent_scan__sliding_block_cached__mixer_s_mlp__decode_kernel(
    A_x, A_k_cache, A_v_cache, A_wq, A_wo, B_x, B_w1, B_w2, B_w3, B_w4, grad_out):
  return _fn(A_x, A_k_cache, A_v_cache, A_wq, A_wo, B_x, B_w1, B_w2, B_w3, B_w4, grad_out)
```

```python
import jax
import jax.numpy as jnp
from jax import lax
import jax.experimental.pallas as pl
import jax.experimental.pallas.tpu as pltpu

B, D, F = 4, 512, 1792
HQ, HKV, SK, DH = 32, 8, 8192, 128
REP = HQ // HKV
SLABS = B * HKV
W = min(4096, max(256, SK // 4))
HALF = SK // 2
ROWS = 8
EPS = 1e-5
BF16, F32 = jnp.bfloat16, jnp.float32

READ_STREAMS = 16
READ_SLOTS = 64
READ_COLS = READ_SLOTS // READ_STREAMS
KV_ROWS = 64

WRITE_ROWS = 56
GROUP = 6
GROUPS = [(GROUP * i, GROUP) for i in range(9)] + [(54, 5), (59, 5)]

assert 2 * W == HALF and 2 * REP == ROWS and B <= ROWS
assert sum(size for _, size in GROUPS) == 2 * SLABS

NN = (((1,), (0,)), ((), ()))
NT = (((1,), (1,)), ((), ()))


def _dot(a, b, dims=NN):
  return lax.dot_general(a.astype(BF16), b.astype(BF16), dims, preferred_element_type=F32)


def _layernorm(x):
  xc = x - jnp.mean(x, axis=-1, keepdims=True)
  rstd = 1.0 / jnp.sqrt(jnp.mean(xc * xc, axis=-1, keepdims=True) + EPS)
  return xc * rstd, rstd


def _layernorm_bwd(dy, y, rstd):
  return rstd * (dy - jnp.mean(dy, axis=-1, keepdims=True)
                 - y * jnp.mean(dy * y, axis=-1, keepdims=True))


def _gelu_and_grad(x):
  c0, c1 = 0.7978845608028654, 0.044715
  x2 = x * x
  t = jnp.tanh(c0 * (x + c1 * x * x2))
  cdf = 0.5 * (1.0 + t)
  return x * cdf, cdf + x * (0.5 * (1.0 - t * t)) * (c0 * (1.0 + 3.0 * c1 * x2))


def _ds(index, size):
  start = index * size
  return pl.ds(start if isinstance(start, int) else pl.multiple_of(start, size), size)


def _head_rows(head, copy=0):
  return pl.ds((head // REP) * ROWS + head % REP + copy * REP, B, stride=HKV * ROWS)


def _scatter_heads(ref, val):
  for head in range(HQ):
    tile = val[:B, head * DH:(head + 1) * DH]
    ref[_head_rows(head, 0), :] = tile
    ref[_head_rows(head, 1), :] = tile


def _gather_heads(ref):
  pad = jnp.zeros((ROWS - B, DH), F32)
  return jnp.concatenate(
      [jnp.concatenate([ref[_head_rows(head), :], pad], axis=0) for head in range(HQ)], axis=1)


def _attention_step(slab, kbuf, vbuf, q_s, do_s, o_s, dq_s):
  rows = _ds(slab, ROWS)
  q, do = q_s[rows, :], do_s[rows, :]
  k, v = kbuf[2 * slab + 1], vbuf[2 * slab + 1]
  scale = DH ** -0.5
  s = _dot(q, k, NT) * scale
  e = jnp.exp(s - jnp.max(s, axis=-1, keepdims=True))
  p = e / jnp.sum(e, axis=-1, keepdims=True)
  dp = _dot(do, v, NT)
  ds = p * (dp - jnp.sum(p * dp, axis=-1, keepdims=True)) * scale
  o_s[rows, :] = _dot(p, v)
  dq_s[rows, :] = _dot(ds, k)
  lhs = jnp.where(lax.broadcasted_iota(jnp.int32, s.shape, 0) < REP, ds, p)
  upper = lax.broadcasted_iota(jnp.int32, q.shape, 0) < REP
  rhs = jnp.concatenate([jnp.where(upper, q, 0.0), jnp.where(upper, 0.0, do)], axis=1)
  dkv = _dot(lhs.T, rhs).astype(BF16)
  kbuf[2 * slab + 1] = dkv[:, :DH]
  vbuf[2 * slab + 1] = dkv[:, DH:]
  kbuf[2 * slab] = jnp.zeros((W, DH), BF16)
  vbuf[2 * slab] = jnp.zeros((W, DH), BF16)


def _kernel(x_hbm, k_hbm, v_hbm, wq_hbm, wo_hbm, w3_hbm, w4_hbm, go_hbm,
            out_hbm, dx_hbm, dk_hbm, dv_hbm, dwq_hbm, dwo_hbm, dw3_hbm, dw4_hbm,
            kbuf, vbuf, wq, wo, w3, w4, dwq, dwo, dw3, dw4, zeros,
            x_s, go_s, out_s, dx_s, q_s, do_s, o_s, dq_s, dv_sem):

  def mlp_chunk(col, s):
    if s % 2 == 0:
      idx = (_ds((s // 2) * 8 + col // 2, 8), _ds(col % 2, F // 2))
      return w3_hbm.at[idx], w3.at[idx]
    if s < READ_STREAMS - 1:
      idx = (_ds((s // 2) * 16 + col, 16), slice(None))
      return w4_hbm.at[idx], w4.at[idx]
    return {0: (x_hbm, x_s), 1: (go_hbm, go_s)}.get(col)

  def proj_chunk(col, s):
    if s % 2 == 0:
      idx = (_ds((s // 2) * 8 + (col >> 2), 8), _ds(col & 3, 1024))
      return wq_hbm.at[idx], wq.at[idx]
    idx = (_ds((s // 2) * 32 + col, 16), slice(None))
    return wo_hbm.at[idx], wo.at[idx]

  def cache_chunk(col, s):
    src, dst = ((k_hbm, kbuf), (v_hbm, vbuf))[s // HKV]
    slab, run = (col >> 5) * HKV + s % HKV, col & 31
    return src.at[slab, _ds((SK - W) // KV_ROWS + run, KV_ROWS)], dst.at[2 * slab + 1, _ds(run, KV_ROWS)]

  def read_everything(start_writes, sems):
    def copy(chunk, window, slot):
      refs = chunk(window * READ_COLS + slot // READ_STREAMS, slot % READ_STREAMS)
      return None if refs is None else pltpu.make_async_copy(*refs, sems.at[slot])

    def start(cp, slot):
      cp.start(priority=0 if slot % 4 == 0 else 1)

    in_flight = [None] * READ_SLOTS
    for chunk, looped, windows in ((mlp_chunk, False, 4), (proj_chunk, True, 8), (cache_chunk, True, 32)):
      for window in range(1 if looped else windows):
        for slot in range(READ_SLOTS):
          cp = copy(chunk, window, slot)
          if cp is not None:
            if in_flight[slot] is not None:
              in_flight[slot].wait()
            start(cp, slot)
            in_flight[slot] = cp
      if looped:
        def next_window(window, carry, chunk=chunk):
          for slot in range(READ_SLOTS):
            copy(chunk, window - 1, slot).wait()
            start(copy(chunk, window, slot), slot)
          return carry
        lax.fori_loop(1, windows, next_window, None)
        in_flight = [copy(chunk, windows - 1, slot) for slot in range(READ_SLOTS)]
      else:
        zeros[...] = jnp.zeros(zeros.shape, BF16)
    for cp in in_flight[:READ_SLOTS // 2]:
      cp.wait()
    start_writes()
    for cp in in_flight[READ_SLOTS // 2:]:
      cp.wait()

  def sweep(copy):
    def column(c, carry):
      copy(pl.multiple_of(c * WRITE_ROWS, 8), WRITE_ROWS)
      return carry
    lax.fori_loop(0, W // WRITE_ROWS, column, None)
    copy(W - W % WRITE_ROWS, W % WRITE_ROWS)

  def write_zeros(dst, sem, first, size):
    sweep(lambda r, n: pltpu.make_async_copy(
        zeros.at[pl.ds(0, size), pl.ds(0, n)], dst.at[pl.ds(first, size), pl.ds(r, n)], sem).start())

  def write_grad(src, dst, sem, first, size):
    sweep(lambda r, n: pltpu.make_async_copy(
        src.at[pl.ds(first, size), pl.ds(r, n)], dst.at[pl.ds(first, size), pl.ds(W + r, n)], sem).start())

  def run(read_sems_shape, sems):
    out_sem, dx_sem, dk_sem, dwq_sem, dwo_sem, dw3_sem, dw4_sem = (sems.at[i] for i in range(7))
    pl.run_scoped(
        lambda read_sems: read_everything(lambda: write_zeros(dk_hbm, dk_sem, *GROUPS[8]), read_sems),
        read_sems_shape)
    write_zeros(dv_hbm, dv_sem, *GROUPS[8])
    write_zeros(dk_hbm, dk_sem, *GROUPS[9])

    pad = jnp.zeros((ROWS - B, D), F32)
    x = jnp.concatenate([x_s[...].astype(F32), pad], axis=0)
    go = jnp.concatenate([go_s[...].astype(F32), pad], axis=0)
    xn, rstd1 = _layernorm(x)
    ln2, rstd2 = _layernorm(xn)
    h, dgelu = _gelu_and_grad(_dot(ln2, w3[...]))
    mix = xn + _dot(h, w4[...])
    sig = jax.nn.sigmoid(mix)
    gate = mix * sig
    dattn = go * gate
    _scatter_heads(q_s, _dot(xn, wq[...]))
    write_zeros(dv_hbm, dv_sem, *GROUPS[9])
    _scatter_heads(do_s, _dot(dattn, wo[...], NT))

    def two_slabs(i, carry):
      first = (i >> 1) * GROUP

      @pl.when((i & 1) == 0)
      def _():
        write_zeros(dk_hbm, dk_sem, first, GROUP)

      @pl.when((i & 1) == 1)
      def _():
        write_zeros(dv_hbm, dv_sem, first, GROUP)

      def step(slab, carry):
        _attention_step(slab, kbuf, vbuf, q_s, do_s, o_s, dq_s)
        return carry
      return lax.fori_loop(2 * i, 2 * i + 2, step, carry)

    lax.fori_loop(0, SLABS // 2, two_slabs, None)

    write_zeros(dk_hbm, dk_sem, *GROUPS[10])
    o, dq = _gather_heads(o_s), _gather_heads(dq_s)
    attn = _dot(o, wo[...])
    out_s[...] = (x + attn * gate)[:B].astype(BF16)
    dmix = go * attn * (sig * (1.0 + mix * (1.0 - sig)))
    dpre = _dot(dmix, w4[...], NT) * dgelu
    dxn = dmix + _layernorm_bwd(_dot(dpre, w3[...], NT), ln2, rstd2) + _dot(dq, wq[...], NT)
    dx_s[...] = (go + _layernorm_bwd(dxn, xn, rstd1))[:B].astype(BF16)
    write_zeros(dv_hbm, dv_sem, *GROUPS[10])
    pltpu.make_async_copy(out_s, out_hbm, out_sem).start()
    pltpu.make_async_copy(dx_s, dx_hbm, dx_sem).start()

    def weight_grad(ref, act, grad):
      bands, rows, _ = ref.shape
      for i in range(bands):
        ref[i] = _dot(act[:, i * rows:(i + 1) * rows].T, grad).astype(BF16)

    pending = [(dwq, xn, dq), (dwo, o, dattn), (dw3, ln2, dpre), (dw4, h, dmix)]
    for i, group in enumerate(GROUPS):
      write_grad(kbuf, dk_hbm, dk_sem, *group)
      if i < len(pending):
        weight_grad(*pending[i])

    def write_wq_w3(c, carry):
      idx = (slice(None), _ds(c >> 2, 8), _ds(c & 3, 1024))
      pltpu.make_async_copy(dwq.at[idx], dwq_hbm.at[idx], dwq_sem).start()
      idx = (slice(None), _ds(c >> 1, 8), _ds(c & 1, F // 2))
      pltpu.make_async_copy(dw3.at[idx], dw3_hbm.at[idx], dw3_sem).start()
      return carry

    def write_wo_w4(c, carry):
      idx = (slice(None), _ds(c, 16), slice(None))
      pltpu.make_async_copy(dwo.at[idx], dwo_hbm.at[idx], dwo_sem).start()

      @pl.when(c < dw4.shape[1] // 16)
      def _():
        pltpu.make_async_copy(dw4.at[idx], dw4_hbm.at[idx], dw4_sem).start()
      return carry

    lax.fori_loop(0, 64, write_wq_w3, None)
    lax.fori_loop(0, 64, write_wo_w4, None)

    for group in GROUPS[:2]:
      write_grad(vbuf, dv_hbm, dv_sem, *group)
    for ref, sem in ((out_hbm, out_sem), (dx_hbm, dx_sem), (dk_hbm, dk_sem), (dwq_hbm, dwq_sem),
                     (dw3_hbm, dw3_sem), (dwo_hbm, dwo_sem), (dw4_hbm, dw4_sem)):
      pltpu.make_async_copy(ref, ref, sem).wait()

  pl.run_scoped(lambda sems: run(pltpu.SemaphoreType.DMA((READ_SLOTS,)), sems),
                pltpu.SemaphoreType.DMA((7,)))
  for group in GROUPS[2:]:
    write_grad(vbuf, dv_hbm, dv_sem, *group)
  pltpu.make_async_copy(dv_hbm, dv_hbm, dv_sem).wait()


@jax.jit
def pallas_recurrent_scan__sliding_block_cached__mixer_s_mlp__decode_kernel(
    A_x: jax.Array,
    A_k_cache: jax.Array,
    A_v_cache: jax.Array,
    A_wq: jax.Array,
    A_wo: jax.Array,
    B_x: jax.Array,
    B_w1: jax.Array,
    B_w2: jax.Array,
    B_w3: jax.Array,
    B_w4: jax.Array,
    grad_out: jax.Array,
):
  del B_x, B_w1, B_w2
  assert A_x.shape == (B, 1, D) and A_k_cache.shape == (B, HKV, SK, DH) and B_w3.shape == (D, F)
  grad_shapes = [(4, D // 4, HQ * DH), (4, HQ * DH // 4, D), (2, D // 2, F), (2, F // 2, D)]
  out_shapes = [(B, D)] * 2 + [(2 * SLABS, HALF, DH)] * 2 + grad_shapes
  hbm = pl.BlockSpec(memory_space=pltpu.HBM)
  out, dx, dk, dv, dwq, dwo, dw3, dw4 = pl.pallas_call(
      _kernel,
      out_shape=[jax.ShapeDtypeStruct(shape, BF16) for shape in out_shapes],
      in_specs=[hbm] * 8,
      out_specs=[hbm] * 8,
      scratch_shapes=(
          [pltpu.VMEM((2 * SLABS, W, DH), BF16)] * 2
          + [pltpu.VMEM(w.shape, BF16) for w in (A_wq, A_wo, B_w3, B_w4)]
          + [pltpu.VMEM(shape, BF16) for shape in grad_shapes]
          + [pltpu.VMEM((GROUP, WRITE_ROWS, DH), BF16)]
          + [pltpu.VMEM((B, D), BF16)] * 4
          + [pltpu.VMEM((SLABS * ROWS, DH), F32)] * 4
          + [pltpu.SemaphoreType.DMA]),
      compiler_params=pltpu.CompilerParams(vmem_limit_bytes=100 * 2**20),
  )(A_x.reshape(B, D), A_k_cache.reshape(SLABS, SK, DH), A_v_cache.reshape(SLABS, SK, DH),
    A_wq, A_wo, B_w3, B_w4, grad_out.reshape(B, D))
  return (out.reshape(A_x.shape), dx.reshape(A_x.shape),
          dk.reshape(A_k_cache.shape), dv.reshape(A_v_cache.shape),
          dwq.reshape(A_wq.shape), dwo.reshape(A_wo.shape),
          dw3.reshape(B_w3.shape), dw4.reshape(B_w4.shape))
```

```python
import jax
import jax.numpy as jnp
from jax import lax
import jax.experimental.pallas as pl
import jax.experimental.pallas.tpu as pltpu

B, D, F = 4, 512, 1792
HQ, HKV, SK, DH = 32, 8, 8192, 128
REP = HQ // HKV
SLABS = B * HKV
W = min(4096, max(256, SK // 4))
HALF = SK // 2
ROWS = 8
EPS = 1e-5
BF16, F32 = jnp.bfloat16, jnp.float32

READ_STREAMS = 16
READ_SLOTS = 64
READ_COLS = READ_SLOTS // READ_STREAMS
KV_ROWS = 64

WRITE_ROWS = 56
GROUP = 6
GROUPS = [(GROUP * i, GROUP) for i in range(9)] + [(54, 5), (59, 5)]

assert 2 * W == HALF and 2 * REP == ROWS and B <= ROWS
assert sum(size for _, size in GROUPS) == 2 * SLABS

NN = (((1,), (0,)), ((), ()))
NT = (((1,), (1,)), ((), ()))


def _dot(a, b, dims=NN):
  return lax.dot_general(a.astype(BF16), b.astype(BF16), dims, preferred_element_type=F32)


def _layernorm(x):
  xc = x - jnp.mean(x, axis=-1, keepdims=True)
  rstd = 1.0 / jnp.sqrt(jnp.mean(xc * xc, axis=-1, keepdims=True) + EPS)
  return xc * rstd, rstd


def _layernorm_bwd(dy, y, rstd):
  return rstd * (dy - jnp.mean(dy, axis=-1, keepdims=True)
                 - y * jnp.mean(dy * y, axis=-1, keepdims=True))


def _gelu_and_grad(x):
  c0, c1 = 0.7978845608028654, 0.044715
  x2 = x * x
  t = jnp.tanh(c0 * (x + c1 * x * x2))
  cdf = 0.5 * (1.0 + t)
  return x * cdf, cdf + x * (0.5 * (1.0 - t * t)) * (c0 * (1.0 + 3.0 * c1 * x2))


def _ds(index, size):
  start = index * size
  return pl.ds(start if isinstance(start, int) else pl.multiple_of(start, size), size)


def _scatter_heads(ref, val):
  for slab in range(SLABS):
    b, kv = divmod(slab, HKV)
    heads = [val[b:b + 1, head * DH:(head + 1) * DH] for head in range(kv * REP, (kv + 1) * REP)]
    ref[slab] = jnp.concatenate(heads + heads, axis=0)


def _gather_heads(ref):
  pad = jnp.zeros((ROWS - B, DH), F32)
  tiles = []
  for head in range(HQ):
    kv, r = divmod(head, REP)
    tiles.append(jnp.concatenate([ref[b * HKV + kv, r:r + 1, :] for b in range(B)] + [pad], axis=0))
  return jnp.concatenate(tiles, axis=1)


def _attention_step(slab, kbuf, vbuf, q_s, do_s, o_s, dq_s):
  q, do = q_s[slab], do_s[slab]
  k, v = kbuf[2 * slab + 1], vbuf[2 * slab + 1]
  scale = DH ** -0.5
  s = _dot(q, k, NT) * scale
  e = jnp.exp(s - jnp.max(s, axis=-1, keepdims=True))
  p = e / jnp.sum(e, axis=-1, keepdims=True)
  dp = _dot(do, v, NT)
  ds = p * (dp - jnp.sum(p * dp, axis=-1, keepdims=True)) * scale
  o_s[slab] = _dot(p, v)
  dq_s[slab] = _dot(ds, k)
  lhs = jnp.where(lax.broadcasted_iota(jnp.int32, s.shape, 0) < REP, ds, p)
  upper = lax.broadcasted_iota(jnp.int32, q.shape, 0) < REP
  rhs = jnp.concatenate([jnp.where(upper, q, 0.0), jnp.where(upper, 0.0, do)], axis=1)
  dkv = _dot(lhs.T, rhs).astype(BF16)
  kbuf[2 * slab + 1] = dkv[:, :DH]
  vbuf[2 * slab + 1] = dkv[:, DH:]
  kbuf[2 * slab] = jnp.zeros((W, DH), BF16)
  vbuf[2 * slab] = jnp.zeros((W, DH), BF16)


def _kernel(x_hbm, k_hbm, v_hbm, wq_hbm, wo_hbm, w3_hbm, w4_hbm, go_hbm,
            out_hbm, dx_hbm, dk_hbm, dv_hbm, dwq_hbm, dwo_hbm, dw3_hbm, dw4_hbm,
            kbuf, vbuf, wq, wo, w3, w4, dwq, dwo, dw3, dw4, zeros,
            x_s, go_s, out_s, dx_s, q_s, do_s, o_s, dq_s, dv_sem):

  def mlp_chunk(col, s):
    if s % 2 == 0:
      idx = (_ds((s // 2) * 8 + col // 2, 8), _ds(col % 2, F // 2))
      return w3_hbm.at[idx], w3.at[idx]
    if s < READ_STREAMS - 1:
      idx = (_ds((s // 2) * 16 + col, 16), slice(None))
      return w4_hbm.at[idx], w4.at[idx]
    return {0: (x_hbm, x_s), 1: (go_hbm, go_s)}.get(col)

  def proj_chunk(col, s):
    if s % 2 == 0:
      idx = (_ds((s // 2) * 8 + (col >> 2), 8), _ds(col & 3, 1024))
      return wq_hbm.at[idx], wq.at[idx]
    idx = (_ds((s // 2) * 32 + col, 16), slice(None))
    return wo_hbm.at[idx], wo.at[idx]

  def cache_chunk(col, s):
    src, dst = ((k_hbm, kbuf), (v_hbm, vbuf))[s // HKV]
    slab, run = (col >> 5) * HKV + s % HKV, col & 31
    return src.at[slab, _ds((SK - W) // KV_ROWS + run, KV_ROWS)], dst.at[2 * slab + 1, _ds(run, KV_ROWS)]

  def read_everything(start_writes, sems):
    def copy(chunk, window, slot):
      refs = chunk(window * READ_COLS + slot // READ_STREAMS, slot % READ_STREAMS)
      return None if refs is None else pltpu.make_async_copy(*refs, sems.at[slot])

    def start(cp, slot):
      cp.start(priority=0 if slot % 4 == 0 else 1)

    in_flight = [None] * READ_SLOTS
    for chunk, looped, windows in ((mlp_chunk, False, 4), (proj_chunk, True, 8), (cache_chunk, True, 32)):
      for window in range(1 if looped else windows):
        for slot in range(READ_SLOTS):
          cp = copy(chunk, window, slot)
          if cp is not None:
            if in_flight[slot] is not None:
              in_flight[slot].wait()
            start(cp, slot)
            in_flight[slot] = cp
      if looped:
        def next_window(window, carry, chunk=chunk):
          for slot in range(READ_SLOTS):
            copy(chunk, window - 1, slot).wait()
            start(copy(chunk, window, slot), slot)
          return carry
        lax.fori_loop(1, windows, next_window, None)
        in_flight = [copy(chunk, windows - 1, slot) for slot in range(READ_SLOTS)]
      else:
        zeros[...] = jnp.zeros(zeros.shape, BF16)
    for cp in in_flight[:READ_SLOTS // 2]:
      cp.wait()
    start_writes()
    for cp in in_flight[READ_SLOTS // 2:]:
      cp.wait()

  def sweep(copy):
    def column(c, carry):
      copy(pl.multiple_of(c * WRITE_ROWS, 8), WRITE_ROWS)
      return carry
    lax.fori_loop(0, W // WRITE_ROWS, column, None)
    copy(W - W % WRITE_ROWS, W % WRITE_ROWS)

  def write_zeros(dst, sem, first, size):
    sweep(lambda r, n: pltpu.make_async_copy(
        zeros.at[pl.ds(0, size), pl.ds(0, n)], dst.at[pl.ds(first, size), pl.ds(r, n)], sem).start())

  def write_grad(src, dst, sem, first, size):
    sweep(lambda r, n: pltpu.make_async_copy(
        src.at[pl.ds(first, size), pl.ds(r, n)], dst.at[pl.ds(first, size), pl.ds(W + r, n)], sem).start())

  def run(read_sems_shape, sems):
    out_sem, dx_sem, dk_sem, dwq_sem, dwo_sem, dw3_sem, dw4_sem = (sems.at[i] for i in range(7))
    pl.run_scoped(
        lambda read_sems: read_everything(lambda: write_zeros(dk_hbm, dk_sem, *GROUPS[8]), read_sems),
        read_sems_shape)
    write_zeros(dv_hbm, dv_sem, *GROUPS[8])
    write_zeros(dk_hbm, dk_sem, *GROUPS[9])

    pad = jnp.zeros((ROWS - B, D), F32)
    x = jnp.concatenate([x_s[...].astype(F32), pad], axis=0)
    go = jnp.concatenate([go_s[...].astype(F32), pad], axis=0)
    xn, rstd1 = _layernorm(x)
    ln2, rstd2 = _layernorm(xn)
    h, dgelu = _gelu_and_grad(_dot(ln2, w3[...]))
    mix = xn + _dot(h, w4[...])
    sig = jax.nn.sigmoid(mix)
    gate = mix * sig
    dattn = go * gate
    _scatter_heads(q_s, _dot(xn, wq[...]))
    write_zeros(dv_hbm, dv_sem, *GROUPS[9])
    _scatter_heads(do_s, _dot(dattn, wo[...], NT))

    def two_slabs(i, carry):
      first = (i >> 1) * GROUP

      @pl.when((i & 1) == 0)
      def _():
        write_zeros(dk_hbm, dk_sem, first, GROUP)

      @pl.when((i & 1) == 1)
      def _():
        write_zeros(dv_hbm, dv_sem, first, GROUP)

      def step(slab, carry):
        _attention_step(slab, kbuf, vbuf, q_s, do_s, o_s, dq_s)
        return carry
      return lax.fori_loop(2 * i, 2 * i + 2, step, carry)

    lax.fori_loop(0, SLABS // 2, two_slabs, None)

    write_zeros(dk_hbm, dk_sem, *GROUPS[10])
    o, dq = _gather_heads(o_s), _gather_heads(dq_s)
    attn = _dot(o, wo[...])
    out_s[...] = (x + attn * gate)[:B].astype(BF16)
    dmix = go * attn * (sig * (1.0 + mix * (1.0 - sig)))
    dpre = _dot(dmix, w4[...], NT) * dgelu
    dxn = dmix + _layernorm_bwd(_dot(dpre, w3[...], NT), ln2, rstd2) + _dot(dq, wq[...], NT)
    dx_s[...] = (go + _layernorm_bwd(dxn, xn, rstd1))[:B].astype(BF16)
    write_zeros(dv_hbm, dv_sem, *GROUPS[10])
    pltpu.make_async_copy(out_s, out_hbm, out_sem).start()
    pltpu.make_async_copy(dx_s, dx_hbm, dx_sem).start()

    def weight_grad(ref, act, grad):
      bands, rows, _ = ref.shape
      for i in range(bands):
        ref[i] = _dot(act[:, i * rows:(i + 1) * rows].T, grad).astype(BF16)

    pending = [(dwq, xn, dq), (dwo, o, dattn), (dw3, ln2, dpre), (dw4, h, dmix)]
    for i, group in enumerate(GROUPS):
      write_grad(kbuf, dk_hbm, dk_sem, *group)
      if i < len(pending):
        weight_grad(*pending[i])

    def write_wq_w3(c, carry):
      idx = (slice(None), _ds(c >> 2, 8), _ds(c & 3, 1024))
      pltpu.make_async_copy(dwq.at[idx], dwq_hbm.at[idx], dwq_sem).start()
      idx = (slice(None), _ds(c >> 1, 8), _ds(c & 1, F // 2))
      pltpu.make_async_copy(dw3.at[idx], dw3_hbm.at[idx], dw3_sem).start()
      return carry

    def write_wo_w4(c, carry):
      idx = (slice(None), _ds(c, 16), slice(None))
      pltpu.make_async_copy(dwo.at[idx], dwo_hbm.at[idx], dwo_sem).start()

      @pl.when(c < dw4.shape[1] // 16)
      def _():
        pltpu.make_async_copy(dw4.at[idx], dw4_hbm.at[idx], dw4_sem).start()
      return carry

    lax.fori_loop(0, 64, write_wq_w3, None)
    lax.fori_loop(0, 64, write_wo_w4, None)

    for group in GROUPS[:2]:
      write_grad(vbuf, dv_hbm, dv_sem, *group)
    for ref, sem in ((out_hbm, out_sem), (dx_hbm, dx_sem), (dk_hbm, dk_sem), (dwq_hbm, dwq_sem),
                     (dw3_hbm, dw3_sem), (dwo_hbm, dwo_sem), (dw4_hbm, dw4_sem)):
      pltpu.make_async_copy(ref, ref, sem).wait()

  pl.run_scoped(lambda sems: run(pltpu.SemaphoreType.DMA((READ_SLOTS,)), sems),
                pltpu.SemaphoreType.DMA((7,)))
  for group in GROUPS[2:]:
    write_grad(vbuf, dv_hbm, dv_sem, *group)
  pltpu.make_async_copy(dv_hbm, dv_hbm, dv_sem).wait()


@jax.jit
def pallas_recurrent_scan__sliding_block_cached__mixer_s_mlp__decode_kernel(
    A_x: jax.Array,
    A_k_cache: jax.Array,
    A_v_cache: jax.Array,
    A_wq: jax.Array,
    A_wo: jax.Array,
    B_x: jax.Array,
    B_w1: jax.Array,
    B_w2: jax.Array,
    B_w3: jax.Array,
    B_w4: jax.Array,
    grad_out: jax.Array,
):
  del B_x, B_w1, B_w2
  assert A_x.shape == (B, 1, D) and A_k_cache.shape == (B, HKV, SK, DH) and B_w3.shape == (D, F)
  grad_shapes = [(4, D // 4, HQ * DH), (4, HQ * DH // 4, D), (2, D // 2, F), (2, F // 2, D)]
  out_shapes = [(B, D)] * 2 + [(2 * SLABS, HALF, DH)] * 2 + grad_shapes
  hbm = pl.BlockSpec(memory_space=pltpu.HBM)
  out, dx, dk, dv, dwq, dwo, dw3, dw4 = pl.pallas_call(
      _kernel,
      out_shape=[jax.ShapeDtypeStruct(shape, BF16) for shape in out_shapes],
      in_specs=[hbm] * 8,
      out_specs=[hbm] * 8,
      scratch_shapes=(
          [pltpu.VMEM((2 * SLABS, W, DH), BF16)] * 2
          + [pltpu.VMEM(w.shape, BF16) for w in (A_wq, A_wo, B_w3, B_w4)]
          + [pltpu.VMEM(shape, BF16) for shape in grad_shapes]
          + [pltpu.VMEM((GROUP, WRITE_ROWS, DH), BF16)]
          + [pltpu.VMEM((B, D), BF16)] * 4
          + [pltpu.VMEM((SLABS, ROWS, DH), F32)] * 4
          + [pltpu.SemaphoreType.DMA]),
      compiler_params=pltpu.CompilerParams(vmem_limit_bytes=100 * 2**20),
  )(A_x.reshape(B, D), A_k_cache.reshape(SLABS, SK, DH), A_v_cache.reshape(SLABS, SK, DH),
    A_wq, A_wo, B_w3, B_w4, grad_out.reshape(B, D))
  return (out.reshape(A_x.shape), dx.reshape(A_x.shape),
          dk.reshape(A_k_cache.shape), dv.reshape(A_v_cache.shape),
          dwq.reshape(A_wq.shape), dwo.reshape(A_wo.shape),
          dw3.reshape(B_w3.shape), dw4.reshape(B_w4.shape))
```
